```python
import os as _os
_os.environ.setdefault("JAX_PLATFORMS", "cpu")
import jax
import jax.numpy as jnp

def _softmax(x, axis=-1):
    return jax.nn.softmax(x, axis=axis)
def _gelu(x):
    return jax.nn.gelu(x, approximate=True)
def _silu(x):
    return jax.nn.silu(x)
def _sigmoid(x):
    return jax.nn.sigmoid(x)
def _layernorm(x, axis=-1, eps=1e-5):
    m = jnp.mean(x, axis=axis, keepdims=True)
    v = jnp.var(x, axis=axis, keepdims=True)
    return (x - m) / jnp.sqrt(v + eps)
def _scatter_add(tgt, idx, src, axis=0):
    return tgt.at[idx].add(src)
def _segment_sum(src, seg, n):
    return jax.ops.segment_sum(src, seg, n)
class _Rng:
    def __init__(self, key):
        self._k = key
    def _next(self):
        self._k, sub = jax.random.split(self._k)
        return sub
    def normal(self, shape):
        return jax.random.normal(self._next(), shape, dtype=jnp.bfloat16)
    def randint(self, lo, hi, shape):
        return jax.random.randint(self._next(), shape, lo, hi, dtype=jnp.int32)
    def uniform(self, shape, lo=0.0, hi=1.0):
        return jax.random.uniform(self._next(), shape, jnp.bfloat16, lo, hi)
    def permutation(self, n):
        return jax.random.permutation(self._next(), n)


kernel_name = 'parallel_sum__grouped_kv_mqa__dense_activation_silu__prompt'

def setup_inputs():
    _rng = _Rng(jax.random.key(int.from_bytes(__import__("os").urandom(4), "little")))
    _w = (lambda a: (lambda t: t.astype(jnp.bfloat16) if jnp.issubdtype(t.dtype, jnp.floating) else t)(jnp.asarray(a)))
    def _A_setup():
        B, S, D, H = 1, 2048, 512, 32
        Dh = D // H
        return {
            "x": _w((lambda *s: _rng.normal(s) * 0.05)(B, S, D)),
            "wq": _w((lambda *s: _rng.normal(s) * 0.05)(D, H * Dh)),
            "wk": _w((lambda *s: _rng.normal(s) * 0.05)(D, Dh)),
            "wv": _w((lambda *s: _rng.normal(s) * 0.05)(D, Dh)),
            "wo": _w((lambda *s: _rng.normal(s) * 0.05)(H * Dh, D)),
        }
    _A_in = _A_setup()

    def _B_setup():
        B, S, D, F = 1, 2048, 512, 1376
        return {
            "x": _w((lambda *s: _rng.normal(s) * 0.05)(B, S, D)),
            "w1": _w((lambda *s: _rng.normal(s) * 0.05)(D, F) * (D ** -0.5)),
            "w2": _w((lambda *s: _rng.normal(s) * 0.05)(F, D) * (F ** -0.5)),
        }
    _B_in = _B_setup()

    return {
        "A_x": _A_in["x"],
        "A_wq": _A_in["wq"],
        "A_wk": _A_in["wk"],
        "A_wv": _A_in["wv"],
        "A_wo": _A_in["wo"],
        "B_x": _B_in["x"],
        "B_w1": _B_in["w1"],
        "B_w2": _B_in["w2"],
    }

def reference(A_x, A_wq, A_wk, A_wv, A_wo, B_x, B_w1, B_w2):
    def _A_ref(x, wq, wk, wv, wo):
        B, S, D = x.shape
        H = 32
        Dh = D // H
        q = (lambda x, *d: x.transpose(*d))((x @ wq).reshape(B, S, H, Dh), 0, 2, 1, 3)
        k = x @ wk
        v = x @ wv
        scores = jnp.einsum("bhqd,bkd->bhqk", q, k) * (Dh ** -0.5)
        p = _softmax(scores, axis=-1)
        o = jnp.einsum("bhqk,bkd->bhqd", p, v)
        return (lambda x, *d: x.transpose(*d))(o, 0, 2, 1, 3).reshape(B, S, H * Dh) @ wo

    def _B_ref(x, w1, w2):
        h = jnp.einsum("bsd,df->bsf", x, w1)
        h = _silu(h)
        out = jnp.einsum("bsf,fd->bsd", h, w2)
        return out

    x = A_x
    xn = _layernorm(x, axis=-1)
    return x + _A_ref(xn, A_wq, A_wk, A_wv, A_wo) + _B_ref(xn, B_w1, B_w2)
```

```python
import functools
import math

import jax
import jax.numpy as jnp
import jax.experimental.pallas as pl
import jax.experimental.pallas.tpu as pltpu

H = 32
EPS = 1e-5
TQ = 512
CK = 128
CF = 256
CX = 256
LOG2E = math.log2(math.e)


def _dot_nt(a, b):
    return jax.lax.dot_general(a, b, (((1,), (1,)), ((), ())), preferred_element_type=jnp.float32)


def _kernel(x_hbm, wq_hbm, wkt_ref, wvt_ref, wo_hbm, w1t_hbm, w2_hbm, o_ref,
            x_ref, wq_ref, wo_ref, w1t_ref, w2_ref,
            xn_ref, k_ref, vt_ref, qt_ref, s_ref, ot_ref, xsem, wsem):
    S, D = x_ref.shape
    dh = D // H
    i = pl.program_id(0)
    bf16, f32 = jnp.bfloat16, jnp.float32

    def x_rows(r):
        return pl.ds(pl.multiple_of(r * CX, CX), CX)

    def x_copy(r):
        return pltpu.make_async_copy(x_hbm.at[x_rows(r), :], x_ref.at[x_rows(r), :], xsem.at[r])

    wq_copy = pltpu.make_async_copy(wq_hbm, wq_ref, wsem.at[0])
    late_copies = [
        pltpu.make_async_copy(src, dst, wsem.at[n + 1])
        for n, (src, dst) in enumerate(((w1t_hbm, w1t_ref), (w2_hbm, w2_ref), (wo_hbm, wo_ref)))
    ]

    @pl.when(i == 0)
    def _():
        for r in range(S // CX):
            x_copy(r).start()
        wq_copy.start()

        def ln_body(r, carry):
            rows = x_rows(r)
            x_copy(r).wait()
            xf = x_ref[rows, :].astype(f32)
            mu = jnp.mean(xf, axis=-1, keepdims=True)
            xc = xf - mu
            var = jnp.mean(xc * xc, axis=-1, keepdims=True)
            xn = (xc * jax.lax.rsqrt(var + EPS)).astype(bf16)
            xn_ref[rows, :] = xn
            k_ref[rows, :] = _dot_nt(xn, wkt_ref[...]).astype(bf16)
            return carry
        jax.lax.fori_loop(0, S // CX, ln_body, 0)
        for c in late_copies:
            c.start()
        vt_ref[...] = _dot_nt(wvt_ref[...], xn_ref[...]).astype(bf16)
        wq_copy.wait()

    rows = pl.ds(pl.multiple_of(i * TQ, TQ), TQ)
    xn = xn_ref[rows, :]
    q = jnp.dot(xn, wq_ref[...], preferred_element_type=f32) * (dh ** -0.5 * LOG2E)
    qt_ref[...] = q.T.astype(bf16)

    nck = S // CK

    def head_rows(h):
        return pl.ds(pl.multiple_of(h * dh, dh), dh)

    def scores_chunk(qh, slot, c, m8):
        s = jnp.dot(k_ref[c * CK:(c + 1) * CK, :], qh, preferred_element_type=f32)
        s_ref[slot, c * CK:(c + 1) * CK, :] = s
        cm = jnp.max(s.reshape(CK // 8, 8, TQ), axis=0)
        return cm if m8 is None else jnp.maximum(m8, cm)

    def probs_chunk(slot, c, m, l8, acc):
        p = jnp.exp2(s_ref[slot, c * CK:(c + 1) * CK, :] - m)
        ls = jnp.sum(p.reshape(CK // 8, 8, TQ), axis=0)
        pv = jnp.dot(vt_ref[:, c * CK:(c + 1) * CK], p.astype(bf16), preferred_element_type=f32)
        return (ls, pv) if l8 is None else (l8 + ls, acc + pv)

    def finish(h, l8, acc):
        l = jnp.sum(l8, axis=0, keepdims=True)
        ot_ref[head_rows(h), :] = acc * (1.0 / l)

    m8 = None
    qh = qt_ref[head_rows(0), :]
    for c in range(nck):
        m8 = scores_chunk(qh, 0, c, m8)

    def head_step(h, slot, m8_cur, has_next=True):
        m = jnp.max(m8_cur, axis=0, keepdims=True)
        qn = qt_ref[head_rows(h + 1), :] if has_next else None
        m8n, l8, acc = None, None, None
        for c in range(nck):
            if has_next:
                m8n = scores_chunk(qn, 1 - slot, c, m8n)
            l8, acc = probs_chunk(slot, c, m, l8, acc)
        finish(h, l8, acc)
        return m8n

    def pair_body(j, m8_cur):
        return head_step(2 * j + 1, 1, head_step(2 * j, 0, m8_cur))

    m8 = jax.lax.fori_loop(0, H // 2 - 1, pair_body, m8)

    @pl.when(i == 0)
    def _():
        for c in late_copies:
            c.wait()

    head_step(H - 1, 1, head_step(H - 2, 0, m8), has_next=False)

    o = ot_ref[...].T.astype(bf16)
    y = jnp.dot(o, wo_ref[...], preferred_element_type=f32)
    F = w2_ref.shape[0]
    for f0 in range(0, F, CF):
        f1 = min(f0 + CF, F)
        hid = _dot_nt(xn, w1t_ref[f0:f1, :])
        hid = (hid * jax.nn.sigmoid(hid)).astype(bf16)
        y = y + jnp.dot(hid, w2_ref[f0:f1, :], preferred_element_type=f32)
    o_ref[...] = (x_ref[rows, :].astype(f32) + y).astype(o_ref.dtype)


@jax.jit
def pallas_parallel_sum__grouped_kv_mqa__dense_activation_silu__prompt_kernel(
    A_x: jax.Array,
    A_wq: jax.Array,
    A_wk: jax.Array,
    A_wv: jax.Array,
    A_wo: jax.Array,
    B_x: jax.Array,
    B_w1: jax.Array,
    B_w2: jax.Array,
):
    del B_x
    B, S, D = A_x.shape
    dh = D // H
    x = A_x.reshape(B * S, D)
    full = lambda a: pl.BlockSpec(a.shape, lambda i: (0,) * a.ndim)
    args = (x, A_wq, A_wk.T, A_wv.T, A_wo, B_w1.T, B_w2)
    hbm = pl.BlockSpec(memory_space=pl.ANY)
    out = pl.pallas_call(
        _kernel,
        grid=(S // TQ,),
        in_specs=[hbm, hbm, full(args[2]), full(args[3]), hbm, hbm, hbm],
        out_specs=pl.BlockSpec((TQ, D), lambda i: (i, 0)),
        out_shape=jax.ShapeDtypeStruct((S, D), A_x.dtype),
        scratch_shapes=[
            *[pltpu.VMEM(args[n].shape, args[n].dtype) for n in (0, 1, 4, 5, 6)],
            pltpu.VMEM((S, D), jnp.bfloat16),
            pltpu.VMEM((S, dh), jnp.bfloat16),
            pltpu.VMEM((dh, S), jnp.bfloat16),
            pltpu.VMEM((D, TQ), jnp.bfloat16),
            pltpu.VMEM((2, S, TQ), jnp.float32),
            pltpu.VMEM((D, TQ), jnp.float32),
            pltpu.SemaphoreType.DMA((S // CX,)),
            pltpu.SemaphoreType.DMA((4,)),
        ],
        compiler_params=pltpu.CompilerParams(
            dimension_semantics=("arbitrary",), vmem_limit_bytes=64 << 20),
    )(*args)
    return out.reshape(B, S, D)
```
